```python
import os as _os
_os.environ.setdefault("JAX_PLATFORMS", "cpu")
import jax
import jax.numpy as jnp

def _softmax(x, axis=-1):
    return jax.nn.softmax(x, axis=axis)
def _gelu(x):
    return jax.nn.gelu(x, approximate=True)
def _silu(x):
    return jax.nn.silu(x)
def _sigmoid(x):
    return jax.nn.sigmoid(x)
def _layernorm(x, axis=-1, eps=1e-5):
    m = jnp.mean(x, axis=axis, keepdims=True)
    v = jnp.var(x, axis=axis, keepdims=True)
    return (x - m) / jnp.sqrt(v + eps)
def _scatter_add(tgt, idx, src, axis=0):
    return tgt.at[idx].add(src)
def _segment_sum(src, seg, n):
    return jax.ops.segment_sum(src, seg, n)
class _Rng:
    def __init__(self, key):
        self._k = key
    def _next(self):
        self._k, sub = jax.random.split(self._k)
        return sub
    def normal(self, shape):
        return jax.random.normal(self._next(), shape, dtype=jnp.bfloat16)
    def randint(self, lo, hi, shape):
        return jax.random.randint(self._next(), shape, lo, hi, dtype=jnp.int32)
    def uniform(self, shape, lo=0.0, hi=1.0):
        return jax.random.uniform(self._next(), shape, jnp.bfloat16, lo, hi)
    def permutation(self, n):
        return jax.random.permutation(self._next(), n)


kernel_name = 'sequential_preLN__mha_block__moe_arch_mod__prompt'

def setup_inputs():
    _rng = _Rng(jax.random.key(int.from_bytes(__import__("os").urandom(4), "little")))
    _w = (lambda a: (lambda t: t.astype(jnp.bfloat16) if jnp.issubdtype(t.dtype, jnp.floating) else t)(jnp.asarray(a)))
    def _A_setup():
        B, S, D, H = 1, 2048, 512, 32
        return {
            "x": _w((lambda *s: _rng.normal(s) * 0.05)(B, S, D)),
            "wqkv": _w((lambda *s: _rng.normal(s) * 0.05)(D, 3 * D)),
            "wo": _w((lambda *s: _rng.normal(s) * 0.05)(D, D)),
        }
    _A_in = _A_setup()

    def _B_setup():
        B, S, D, F, C = 1, 2048, 512, 1792, 2
        return {
            "x": _w((lambda *s: _rng.normal(s) * 0.05)(B, S, D)),
            "w_r": _w((lambda *s: _rng.normal(s) * 0.05)(D)),
            "w_gate": _w((lambda *s: _rng.normal(s) * 0.05)(D, F)),
            "w_up": _w((lambda *s: _rng.normal(s) * 0.05)(D, F)),
            "w_down": _w((lambda *s: _rng.normal(s) * 0.05)(F, D)),
        }
    _B_in = _B_setup()

    return {
        "A_x": _A_in["x"],
        "A_wqkv": _A_in["wqkv"],
        "A_wo": _A_in["wo"],
        "B_x": _B_in["x"],
        "B_w_r": _B_in["w_r"],
        "B_w_gate": _B_in["w_gate"],
        "B_w_up": _B_in["w_up"],
        "B_w_down": _B_in["w_down"],
    }

def reference(A_x, A_wqkv, A_wo, B_x, B_w_r, B_w_gate, B_w_up, B_w_down):
    def _A_ref(x, wqkv, wo):
        B, S, D = x.shape
        H = 32
        Dh = D // H
        qkv = (lambda x, *d: x.transpose(*d))((x @ wqkv).reshape(B, S, 3, H, Dh), 2, 0, 3, 1, 4)
        q, k, v = qkv[0], qkv[1], qkv[2]
        scores = jnp.einsum("bhqd,bhkd->bhqk", q, k) * (Dh ** -0.5)
        p = _softmax(scores, axis=-1)
        o = jnp.einsum("bhqk,bhkd->bhqd", p, v)
        return (lambda x, *d: x.transpose(*d))(o, 0, 2, 1, 3).reshape(B, S, D) @ wo

    def _B_ref(x, w_r, w_gate, w_up, w_down):
        B, S, D = x.shape
        C = 2
        r = x @ w_r
        idx = jnp.argsort(-r, axis=-1)[:, :C]
        idx_e = jnp.repeat(idx.reshape(B, C, 1), D, axis=2)
        x_sel = jnp.take_along_axis(x, idx_e, axis=1)
        g = _silu(x_sel @ w_gate)
        u = x_sel @ w_up
        y = (g * u) @ w_down
        r_sel = _sigmoid(jnp.take_along_axis(r, idx, axis=1))
        y = y * r_sel.reshape(B, C, 1)
        b_off = (jnp.arange(B) * S).reshape(B, 1)
        flat_idx = (idx + b_off).reshape(B * C)
        zero = (x * 0.0).reshape(B * S, D)
        upd = _scatter_add(zero, flat_idx, y.reshape(B * C, D), axis=0)
        return x + upd.reshape(B, S, D)

    x = A_x
    h = x + _A_ref(_layernorm(x, axis=-1), A_wqkv, A_wo)
    h2 = h + _B_ref(_layernorm(h, axis=-1), B_w_r, B_w_gate, B_w_up, B_w_down)
    return h2
```

```python
import functools
import jax
import jax.numpy as jnp
from jax import lax
import jax.experimental.pallas as pl
import jax.experimental.pallas.tpu as pltpu

S = 2048
D = 512
H = 32
DH = 16
F = 1792
EPS = 1e-5
LOG2E = 1.4426950408889634
QSCALE = (DH ** -0.5) * LOG2E

TQ = 512
KC = 128
PK = 512
NQ = S // TQ
NIT = H * NQ
UN = 2
RC = 256
L_MIN = 2.0 ** -40

bf16 = jnp.bfloat16
f32 = jnp.float32
u32 = jnp.uint32


def _tobf(x):
    return pltpu.bitcast(x, bf16)


def _tou(x):
    return pltpu.bitcast(x, u32)


def _ln(x):
    m = jnp.mean(x, axis=-1, keepdims=True)
    c = x - m
    v = jnp.mean(c * c, axis=-1, keepdims=True)
    return c * lax.rsqrt(v + EPS)


def _kernel(x_hbm, wqkv_hbm, wo_hbm, wr_hbm, wg_hbm, wu_hbm, wd_hbm, out_hbm,
            x_v, wqkv_v, wo_v, wr_v, wg_v, wu_v, wd_v, out_v,
            wqvt_v, k_v, qt_v, vt_v, kmax_v, kcol_v, p0_v, p1_v, l0_v, l1_v, ot_v, lmin_v, h_v, r_v,
            z_s, sem_x, sem_w, sem_o):
    NXC = S // RC
    x_cp = [pltpu.make_async_copy(x_hbm.at[pl.ds(c * RC, RC)], x_v.at[pl.ds(c * RC, RC)], sem_x.at[c])
            for c in range(NXC)]
    w_cp = [pltpu.make_async_copy(src, dst, sem_w.at[i]) for i, (src, dst) in enumerate(
        [(wqkv_hbm, wqkv_v), (wo_hbm, wo_v), (wr_hbm, wr_v), (wg_hbm, wg_v), (wu_hbm, wu_v), (wd_hbm, wd_v)])]
    w_cp[0].start()
    for c in range(NXC):
        x_cp[c].start()
    for i in range(1, 6):
        w_cp[i].start()
    z_s[0] = 0

    w_cp[0].wait()
    wq_t = wqkv_v[:, 0:D].astype(f32).T
    wv_t = wqkv_v[:, 2 * D:3 * D].astype(f32).T
    wqvt_v[0:D // 2, :] = _tou(wq_t.astype(bf16))
    wqvt_v[D // 2:D, :] = _tou(wv_t.astype(bf16))

    kmax = jnp.zeros((8, D), f32)
    for c in range(NXC):
        x_cp[c].wait()
        ln = _ln(x_v[c * RC:(c + 1) * RC, :].astype(f32)).astype(bf16)
        kc = jnp.dot(ln, wqkv_v[:, D:2 * D], preferred_element_type=f32).astype(bf16)
        for g in range(4):
            k_v[g, c * RC // 2:(c + 1) * RC // 2, :] = _tou(kc[:, g * 128:(g + 1) * 128])
        kmax = jnp.maximum(kmax, jnp.max(jnp.abs(kc.astype(f32)).reshape(RC // 8, 8, D), axis=0))
        qv = lax.dot_general(_tobf(wqvt_v[...]), ln, (((1,), (1,)), ((), ())),
                             preferred_element_type=f32)
        qt_v[:, c * RC:(c + 1) * RC] = _tou((qv[0:D] * QSCALE).astype(bf16))
        vt_v[:, c * RC:(c + 1) * RC] = _tou(qv[D:2 * D].astype(bf16))
    kmax_row = jnp.max(kmax, axis=0, keepdims=True)
    kcol_v[...] = jnp.broadcast_to(kmax_row, (128, D)).T

    p1_v[...] = jnp.zeros_like(p1_v)
    l1_v[...] = jnp.ones_like(l1_v)
    lmin_v[...] = jnp.full(lmin_v.shape, 1.0, f32)

    def step(it, pc_ref, lc_ref, pp_ref, lp_ref):
        z = z_s[0]
        sit = jnp.minimum(it, NIT - 1)
        pit = jnp.clip(it - 1, 0, NIT - 1)
        h = sit % H
        qi = sit // H
        g = h // 8
        hh = h % 8
        q0 = pl.multiple_of(qi * TQ, TQ)
        ph = pit % H
        pq0 = pl.multiple_of((pit // H) * TQ, TQ)
        q16 = qt_v[pl.ds(pl.multiple_of(h * 8, 8), 8), pl.ds(q0, TQ)]
        zero = jnp.zeros_like(q16)
        w = _tobf(jnp.concatenate([jnp.where(hh == j, q16, zero) for j in range(8)], axis=0))
        kcol = kcol_v[pl.ds(pl.multiple_of(h * 16, 16), 16), :]
        aq = jnp.abs(_tobf(q16).astype(f32))
        m = jnp.sum(aq * jnp.concatenate([kcol] * (TQ // 128), axis=1), axis=0, keepdims=True)
        nacc = TQ // 128
        accs = [jnp.zeros((16, 128), f32) for _ in range(nacc)]
        l = jnp.zeros((8, TQ), f32)
        pv = [(kb, nb) for kb in range(S // PK) for nb in range(nacc)]
        nchunks = S // KC
        per = len(pv) // nchunks
        for kc in range(nchunks):
            kk = _tobf(k_v[g, pl.ds(kc * KC // 2, KC // 2), :])
            s = jnp.dot(kk, w, preferred_element_type=f32)
            p = jnp.exp2(s - m)
            l = l + jnp.sum(p.reshape(KC // 8, 8, TQ), axis=0)
            pc_ref[pl.ds(kc * KC // 2, KC // 2), :] = _tou(p.astype(bf16))
            for (kb, nb) in pv[kc * per:(kc + 1) * per]:
                pt = _tobf(pp_ref[pl.ds(pl.multiple_of(z + kb * PK // 2, 8), PK // 2), pl.ds(nb * 128, 128)])
                vt = _tobf(vt_v[pl.ds(pl.multiple_of(ph * 8, 8), 8), pl.ds(kb * PK, PK)])
                accs[nb] = accs[nb] + jnp.dot(vt, pt, preferred_element_type=f32)
        lsum = jnp.sum(lp_ref[...], axis=0, keepdims=True)
        lmin_v[...] = jnp.minimum(lmin_v[...], lsum)
        acc = jnp.concatenate(accs, axis=1)
        ot_v[pl.ds(pl.multiple_of(ph * 8, 8), 8), pl.ds(pq0, TQ)] = _tou((acc / lsum).astype(bf16))
        lc_ref[...] = l

    def body(i, c):
        for u in range(UN // 2):
            step(UN * i + 2 * u, p0_v, l0_v, p1_v, l1_v)
            step(UN * i + 2 * u + 1, p1_v, l1_v, p0_v, l0_v)
        return c

    lax.fori_loop(0, NIT // UN + 1, body, 0)

    @pl.when(jnp.logical_not(jnp.min(lmin_v[...]) >= L_MIN))
    def _():
        TF = 128

        def fb(it, c):
            h = it % H
            q0 = pl.multiple_of((it // H) * TF, TF)
            g = h // 8
            hh = h % 8
            q16 = qt_v[pl.ds(pl.multiple_of(h * 8, 8), 8), pl.ds(q0, TF)]
            zero = jnp.zeros_like(q16)
            w = _tobf(jnp.concatenate([jnp.where(hh == j, q16, zero) for j in range(8)], axis=0))
            s = jnp.dot(_tobf(k_v[g]), w, preferred_element_type=f32)
            p = jnp.exp2(s - jnp.max(s, axis=0, keepdims=True))
            l = jnp.sum(p, axis=0, keepdims=True)
            vt = _tobf(vt_v[pl.ds(pl.multiple_of(h * 8, 8), 8), :])
            o = jnp.dot(vt, p.astype(bf16), preferred_element_type=f32)
            ot_v[pl.ds(pl.multiple_of(h * 8, 8), 8), pl.ds(q0, TF)] = _tou((o / l).astype(bf16))
            return c

        lax.fori_loop(0, H * (S // TF), fb, 0)

    w_cp[1].wait()
    w_cp[2].wait()
    o_cp = [pltpu.make_async_copy(out_v.at[pl.ds(c * RC, RC)], out_hbm.at[pl.ds(c * RC, RC)], sem_o.at[c])
            for c in range(NXC)]
    wr8 = jnp.broadcast_to(wr_v[...], (16, D))
    for c in range(NXC):
        ot = _tobf(ot_v[:, c * RC:(c + 1) * RC])
        attn = lax.dot_general(ot, wo_v[...], (((0,), (0,)), ((), ())), preferred_element_type=f32)
        h = x_v[c * RC:(c + 1) * RC, :].astype(f32) + attn
        h_v[c * RC:(c + 1) * RC, :] = h
        ln2 = _ln(h)
        out_v[c * RC:(c + 1) * RC, :] = (h + ln2).astype(bf16)
        o_cp[c].start()
        r = lax.dot_general(wr8, ln2.astype(bf16), (((1,), (1,)), ((), ())), preferred_element_type=f32)
        r_v[:, c * RC:(c + 1) * RC] = r[0:8]

    r = r_v[0:1, :]
    pos = lax.broadcasted_iota(jnp.int32, (1, S), 1)
    m1 = jnp.max(r)
    i1 = jnp.min(jnp.where(r == m1, pos, S))
    r2 = jnp.where(pos == i1, -jnp.inf, r)
    m2 = jnp.max(r2)
    i2 = jnp.min(jnp.where(r2 == m2, pos, S))
    i1 = jnp.clip(i1, 0, S - 1)
    i2 = jnp.clip(i2, 0, S - 1)
    h1 = h_v[pl.ds(i1, 1), :]
    h2 = h_v[pl.ds(i2, 1), :]
    row = lax.broadcasted_iota(jnp.int32, (16, D), 0)
    hsel = jnp.where(row == 0, h1, h2)
    xsel = _ln(hsel).astype(bf16)
    w_cp[3].wait()
    w_cp[4].wait()
    w_cp[5].wait()
    g = jnp.dot(xsel, wg_v[...], preferred_element_type=f32)
    u = jnp.dot(xsel, wu_v[...], preferred_element_type=f32)
    a = (g * jax.nn.sigmoid(g) * u).astype(bf16)
    y = jnp.dot(a, wd_v[...], preferred_element_type=f32)
    gate = jax.nn.sigmoid(jnp.where(row == 0, m1, m2))
    y = y * gate
    y1 = y[0:1]
    y2 = y[1:2]
    for c in range(NXC):
        o_cp[c].wait()
    for j, idx in enumerate((i1, i2)):
        b0 = pl.multiple_of((idx // 16) * 16, 16)
        hb = h_v[pl.ds(b0, 16), :]
        rows = row + b0
        upd = jnp.where(rows == i1, y1, 0.0) + jnp.where(rows == i2, y2, 0.0)
        out_v[pl.ds(b0, 16), :] = (hb + _ln(hb) + upd).astype(bf16)
        cp = pltpu.make_async_copy(out_v.at[pl.ds(b0, 16)], out_hbm.at[pl.ds(b0, 16)], sem_o.at[j])
        cp.start()
        cp.wait()


@jax.jit
def pallas_sequential_preLN__mha_block__moe_arch_mod__prompt_kernel(A_x, A_wqkv, A_wo, B_x, B_w_r, B_w_gate, B_w_up, B_w_down):
    del B_x
    x = A_x.reshape(S, D)
    wr = B_w_r.reshape(1, D)
    NXC = S // RC
    any_spec = pl.BlockSpec(memory_space=pl.ANY)
    out = pl.pallas_call(
        _kernel,
        out_shape=jax.ShapeDtypeStruct((S, D), bf16),
        in_specs=[any_spec] * 7,
        out_specs=any_spec,
        scratch_shapes=[
            pltpu.VMEM((S, D), bf16),
            pltpu.VMEM((D, 3 * D), bf16),
            pltpu.VMEM((D, D), bf16),
            pltpu.VMEM((1, D), bf16),
            pltpu.VMEM((D, F), bf16),
            pltpu.VMEM((D, F), bf16),
            pltpu.VMEM((F, D), bf16),
            pltpu.VMEM((S, D), bf16),
            pltpu.VMEM((D, D), u32),
            pltpu.VMEM((4, S // 2, 128), u32),
            pltpu.VMEM((D // 2, S), u32),
            pltpu.VMEM((D // 2, S), u32),
            pltpu.VMEM((8, D), f32),
            pltpu.VMEM((D, 128), f32),
            pltpu.VMEM((S // 2, TQ), u32),
            pltpu.VMEM((S // 2, TQ), u32),
            pltpu.VMEM((8, TQ), f32),
            pltpu.VMEM((8, TQ), f32),
            pltpu.VMEM((D // 2, S), u32),
            pltpu.VMEM((1, TQ), f32),
            pltpu.VMEM((S, D), f32),
            pltpu.VMEM((8, S), f32),
            pltpu.SMEM((1,), jnp.int32),
            pltpu.SemaphoreType.DMA((NXC,)),
            pltpu.SemaphoreType.DMA((6,)),
            pltpu.SemaphoreType.DMA((NXC,)),
        ],
        compiler_params=pltpu.CompilerParams(vmem_limit_bytes=100 * 1024 * 1024),
    )(x, A_wqkv, A_wo, wr, B_w_gate, B_w_up, B_w_down)
    return out.reshape(1, S, D)
```

```python
import functools

import jax
import jax.numpy as jnp
from jax import lax
import jax.experimental.pallas as pl
import jax.experimental.pallas.tpu as pltpu

S = 2048
D = 512
H = 32
DH = 16
F = 1792
EPS = 1e-5
QSCALE = (DH ** -0.5) * 1.4426950408889634

TQ = 512
KC = 256
PK = 512
NIT = H * (S // TQ)
UN = 14
LAG = 4
RC = 256
LNR = 64
TC = 128
OC = 128
OUT_GROUPS = ((0, 1024), (1024, 1792), (1792, 2048))

L_MIN = 2.0 ** -60
QK_MAX = 20.0
MAGIC = 12582912.0

bf16 = jnp.bfloat16
f32 = jnp.float32
u32 = jnp.uint32
i32 = jnp.int32
i8 = jnp.int8


def _tobf(x):
    return pltpu.bitcast(x, bf16)


def _toi8(x):
    return pltpu.bitcast(x, i8)


def _tou(x):
    return pltpu.bitcast(x, u32)


def _ln_stats(x):
    m = jnp.sum(x, axis=-1, keepdims=True) * (1.0 / D)
    ms = jnp.sum(x * x, axis=-1, keepdims=True) * (1.0 / D)
    return m, lax.rsqrt(jnp.maximum(ms - m * m, 0.0) + EPS)


def _limbs(t):
    hi = t + MAGIC
    lo = (t - (hi - MAGIC)) * 16.0 + MAGIC
    top = t * 0.0625 + MAGIC
    return hi, lo, top


def _pack8(x):
    return _tou(pltpu.bitcast(x, i32).astype(i8))


_NT = (((1,), (1,)), ((), ()))
_TN = (((0,), (0,)), ((), ()))


def _kernel(x_hbm, wqkv_hbm, wo_hbm, wr_hbm, wg_hbm, wu_hbm, wd_hbm, out_hbm,
            x_v, wq_v, wk_v, wv_v, wo_v, wr_v, wg_v, wu_v, wd_v, out_v,
            wqt_v, wvt_v, ln_v, kf_v, k8_v, w8_v, a_v, vt_v, l0_v, l1_v, ot_v, lmin_v,
            base_v, ln2_v, fix_v, z_s, sem_x, sem_w, sem_o, *p_v):
    nxc = S // RC
    x_cp = [pltpu.make_async_copy(x_hbm.at[pl.ds(c * RC, RC)], x_v.at[pl.ds(c * RC, RC)], sem_x.at[c])
            for c in range(nxc)]
    w_cp = [pltpu.make_async_copy(src, dst, sem_w.at[i]) for i, (src, dst) in enumerate(
        [(wqkv_hbm.at[:, pl.ds(D, D)], wk_v), (wqkv_hbm.at[:, pl.ds(0, D)], wq_v),
         (wqkv_hbm.at[:, pl.ds(2 * D, D)], wv_v),
         (wo_hbm, wo_v), (wr_hbm, wr_v), (wg_hbm, wg_v), (wu_hbm, wu_v), (wd_hbm, wd_v)])]
    x_cp[0].start()
    w_cp[0].start()
    for cp in x_cp[1:] + w_cp[1:]:
        cp.start()
    z_s[0] = 0

    def ln_rows(r0, n):
        for r in range(r0, r0 + n, LNR):
            x = x_v[r:r + LNR, :].astype(f32)
            m, rs = _ln_stats(x)
            ln_v[r // 2:(r + LNR) // 2, :] = _tou(((x - m) * rs).astype(bf16))

    waits = {0: [x_cp[1]], 1: x_cp[2:4], 3: x_cp[4:], nxc - 2: w_cp[1:3]}
    x_cp[0].wait()
    ln_rows(0, RC)
    w_cp[0].wait()
    kmax = jnp.zeros((8, D), f32)
    for c in range(nxc):
        r0 = c * RC
        for cp in waits.get(c, []):
            cp.wait()
        kc = jnp.dot(_tobf(ln_v[r0 // 2:(r0 + RC) // 2, :]), wk_v[...], preferred_element_type=f32)
        kf_v[r0:r0 + RC, :] = kc
        kmax = jnp.maximum(kmax, jnp.max(jnp.abs(kc).reshape(RC // 8, 8, D), axis=0))
        for h in range(H + 1):
            w8_v[32 * h:32 * h + 16, r0:r0 + RC] = jnp.zeros((16, RC), u32)
        if c + 1 < nxc:
            ln_rows(r0 + RC, RC)
        else:
            wqt_v[...] = _tou(wq_v[...].astype(f32).T.astype(bf16))
            wvt_v[...] = _tou(wv_v[...].astype(f32).T.astype(bf16))
    kmax_row = jnp.max(kmax, axis=0, keepdims=True)
    kcol = jnp.broadcast_to(kmax_row, (128, D)).T
    khead = jnp.maximum(jnp.max(kcol.reshape(H, DH, 128), axis=1), 1e-30)
    kinv_col = jnp.broadcast_to((127.0 / khead)[:, None, :], (H, DH, 128)).reshape(D, 128)
    kinv_row = kinv_col.T[0:8, :]

    lane = lax.broadcasted_iota(i32, (8, 128), 1)
    odd16 = (lane & 16) != 0
    odd32 = (lane & 32) != 0
    umax = jnp.minimum(kmax_row * kinv_row + 1.0, 127.0).astype(i32).astype(u32) * jnp.uint32(0x01010101)
    um_e = [pltpu.roll(umax[:, g * 128:(g + 1) * 128], 16, 1) for g in range(4)]
    um_o = [pltpu.roll(umax[:, g * 128:(g + 1) * 128], 112, 1) for g in range(4)]
    never = z_s[0] != 0

    def k_limbs(r0, pace):
        for g in range(4):
            kinv = jnp.where(never, pace, kinv_row[:, g * 128:(g + 1) * 128])
            u = (kf_v[r0:r0 + 32, g * 128:(g + 1) * 128].reshape(4, 8, 128) * kinv).reshape(32, 128)
            hi, lo, top = [_pack8(t) for t in _limbs(u)]
            e1 = jnp.where(odd16, pltpu.roll(lo, 16, 1), hi)
            o1 = jnp.where(odd16, hi, pltpu.roll(lo, 112, 1))
            e2 = jnp.where(odd16, um_e[g], top)
            o2 = jnp.where(odd16, top, um_o[g])
            rs = pl.ds(r0 // 4, 8)
            k8_v[4 * g + 0, rs, :] = jnp.where(odd32, pltpu.roll(e2, 32, 1), e1)
            k8_v[4 * g + 1, rs, :] = jnp.where(odd32, e1, pltpu.roll(e2, 96, 1))
            k8_v[4 * g + 2, rs, :] = jnp.where(odd32, pltpu.roll(o2, 32, 1), o1)
            k8_v[4 * g + 3, rs, :] = jnp.where(odd32, o1, pltpu.roll(o2, 96, 1))

    def q_limbs(c, g, qt):
        cols = slice(c * TC, (c + 1) * TC)
        qs = [qt[j * DH:(j + 1) * DH] for j in range(8)]
        ms = [jnp.maximum(jnp.abs(q[0:8]), jnp.abs(q[8:16])) for q in qs]
        for sh in (4, 2, 1):
            ms = [jnp.maximum(m, pltpu.roll(m, sh, 0)) for m in ms]
        ms = [jnp.maximum(m, 1e-30) for m in ms]
        invs = [pl.reciprocal(m, approx=True) for m in ms]
        invs = [inv * (254.0 - 127.0 * (m * inv)) for m, inv in zip(ms, invs)]
        for j in range(8):
            h = 8 * g + j
            a_v[h:h + 1, cols] = ms[j][j:j + 1]
            t = qs[j] * jnp.concatenate([invs[j], invs[j]], axis=0)
            hi, lo, top = _limbs(t)
            neg = MAGIC - jnp.abs(t)
            x1 = [hi, top] if j % 2 == 0 else [top, hi]
            x2 = [lo, neg] if j % 2 == 0 else [neg, lo]
            blocks = x1 + x2 if (j // 2) % 2 == 0 else x2 + x1
            w8_v[32 * h + 16:32 * h + 32, cols] = _pack8(jnp.concatenate(blocks, axis=0))

    def proj_t(w_ref, g, c):
        ln = _tobf(ln_v[c * TC // 2:(c + 1) * TC // 2, :])
        return lax.dot_general(_tobf(w_ref[64 * g:64 * (g + 1), :]), ln, _NT, preferred_element_type=f32)

    todo = None
    for c in range(S // TC):
        for g in range(4):
            qt = proj_t(wqt_v, g, c)
            if todo is not None:
                todo()
            todo = functools.partial(q_limbs, c, g, qt)
        for g in range(4):
            vt = proj_t(wvt_v, g, c)
            todo()
            vt_v[64 * g:64 * (g + 1), c * TC:(c + 1) * TC] = _tou(vt.astype(bf16))
            todo = functools.partial(k_limbs, c * TC + g * 32, vt[0:8])
    todo()
    a_all = a_v[...] * jnp.concatenate([khead * (QSCALE / (127.0 * 127.0))] * (S // 128), axis=1)
    a_v[...] = a_all
    qk = jnp.max(a_all) * (127.0 * 127.0)

    lmin_v[...] = jnp.full(lmin_v.shape, 1.0, f32)
    nkb = S // PK
    bufs = [(p_v[:nkb], l0_v), (p_v[nkb:], l1_v)]
    hist = []

    def step(sit, pit, cur, prev):
        z = z_s[0]
        if sit is not None:
            h = sit % H
            hh = h % 8
            kidx = (h // 8) * 4 + (hh & 1) * 2 + ((hh >> 1) & 1)
            q0 = pl.multiple_of((sit // H) * TQ, TQ)
            w0 = pl.multiple_of(32 * h + jnp.where(hh >= 4, 0, 16), 16)
            a = a_v[pl.ds(h, 1), pl.ds(q0, TQ)]
            l = jnp.zeros((8, TQ), f32)
        if pit is not None:
            pr0 = pl.multiple_of((pit % H) * 8, 8)
            pq0 = pl.multiple_of((pit // H) * TQ, TQ)
            accs = [jnp.zeros((16, 128), f32) for _ in range(TQ // 128)]
        pv = [(kb, nb) for kb in range(nkb) for nb in range(TQ // 128)]
        per = len(pv) // (S // KC)
        for kc in range(S // KC):
            if sit is not None:
                kk = _toi8(k8_v[kidx, pl.ds(kc * KC // 4, KC // 4), :])
                w = w8_v[pl.ds(w0, 32), pl.ds(q0, TQ)]
                if len(hist) >= LAG:
                    dep = _tou(hist[-LAG][0:8] + hist[-LAG + 1][0:8])
                    dep = jnp.concatenate([dep] * (TQ // 128), axis=1)
                    w = jnp.concatenate([w[0:24], jnp.where(z != 0, dep, w[24:32])], axis=0)
                s = jnp.dot(kk, _toi8(w), preferred_element_type=i32)
                p = jnp.exp2(s.astype(f32) * a)
                cur[0][kc * KC // PK][pl.ds((kc * KC % PK) // 2, KC // 2), :] = _tou(p.astype(bf16))
                l = l + jnp.sum(p.reshape(KC // 8, 8, TQ), axis=0)
            if pit is not None:
                for kb, nb in pv[kc * per:(kc + 1) * per]:
                    pt = _tobf(prev[0][kb][pl.ds(pl.multiple_of(z, 8), PK // 2), pl.ds(nb * 128, 128)])
                    vt = _tobf(vt_v[pl.ds(pr0, 8), pl.ds(kb * PK, PK)])
                    res = jnp.dot(vt, pt, preferred_element_type=f32)
                    hist.append(res)
                    accs[nb] = accs[nb] + res
        if pit is not None:
            lsum = jnp.sum(prev[1][...], axis=0, keepdims=True)
            lmin_v[...] = jnp.minimum(lmin_v[...], lsum)
            o = jnp.concatenate(accs, axis=1) / lsum
            ot_v[pl.ds(pr0, 8), pl.ds(pq0, TQ)] = _tou(o.astype(bf16))
        if sit is not None:
            cur[1][...] = l

    npeel = (NIT - 1) % UN
    step(jnp.int32(0), None, bufs[0], None)
    for i in range(npeel):
        step(jnp.int32(i + 1), jnp.int32(i), bufs[(i + 1) % 2], bufs[i % 2])

    def body(it, carry):
        hist.clear()
        for u in range(npeel, npeel + UN):
            step(UN * it + u + 1, UN * it + u, bufs[(u + 1) % 2], bufs[u % 2])
        hist.clear()
        return carry

    lax.fori_loop(0, (NIT - 1) // UN, body, 0)
    step(None, jnp.int32(NIT - 1), None, bufs[(NIT - 1) % 2])

    ok = jnp.logical_and(jnp.min(lmin_v[...]) >= L_MIN, qk <= QK_MAX)

    @pl.when(jnp.logical_not(ok))
    def _():
        tf = 128

        def fb(it, carry):
            h = it % H
            r8 = pl.multiple_of(h * 8, 8)
            q0 = pl.multiple_of((it // H) * tf, tf)
            lnq = _tobf(ln_v[pl.ds(pl.multiple_of(q0 // 2, tf // 2), tf // 2), :])
            q16 = lax.dot_general(_tobf(wqt_v[pl.ds(r8, 8), :]), lnq, _NT, preferred_element_type=f32)
            q16 = _tou((q16 * QSCALE).astype(bf16))
            zero = jnp.zeros_like(q16)
            w = _tobf(jnp.concatenate([jnp.where(h % 8 == j, q16, zero) for j in range(8)], axis=0))
            kg = kf_v[:, pl.ds(pl.multiple_of((h // 8) * 128, 128), 128)].astype(bf16)
            s = jnp.dot(kg, w, preferred_element_type=f32)
            p = jnp.exp2(s - jnp.max(s, axis=0, keepdims=True))
            l = jnp.sum(p, axis=0, keepdims=True)
            o = jnp.dot(_tobf(vt_v[pl.ds(r8, 8), :]), p.astype(bf16), preferred_element_type=f32)
            ot_v[pl.ds(r8, 8), pl.ds(q0, tf)] = _tou((o / l).astype(bf16))
            return carry

        lax.fori_loop(0, H * (S // tf), fb, 0)

    for cp in w_cp[3:]:
        cp.wait()
    o_cp = [pltpu.make_async_copy(out_v.at[pl.ds(a, b - a)], out_hbm.at[pl.ds(a, b - a)], sem_o.at[j])
            for j, (a, b) in enumerate(OUT_GROUPS)]
    wr = wr_v[...].astype(f32)
    wr_sum = jnp.sum(wr, axis=-1, keepdims=True)
    imin = jnp.int32(-2 ** 31)
    marks = []

    def out_proj(c):
        ot = ot_v[:, c * OC:(c + 1) * OC]
        if c >= 3:
            dep = jnp.broadcast_to(_tou(marks[c - 3]), (8, OC))
            ot = jnp.concatenate([jnp.where(z_s[0] != 0, dep, ot[0:8]), ot[8:]], axis=0)
        return lax.dot_general(_tobf(ot), wo_v[...], _TN, preferred_element_type=f32)

    attn = out_proj(0)
    best1 = jnp.full((8, 1), imin, i32)
    best2 = jnp.full((8, 1), imin, i32)
    for c in range(S // OC):
        r0 = c * OC
        nxt = out_proj(c + 1) if r0 + OC < S else None
        h = x_v[r0:r0 + OC, :].astype(f32) + attn
        m, rs = _ln_stats(h)
        hw = jnp.sum(h * wr, axis=-1, keepdims=True)
        ln2 = (h - m) * rs
        base = h + ln2
        ln2_v[r0:r0 + OC, :] = ln2
        base_v[r0:r0 + OC, :] = base
        out_v[r0:r0 + OC, :] = base.astype(bf16)
        bits = pltpu.bitcast((hw - m * wr_sum) * rs, i32)
        key = jnp.where(bits < 0, bits ^ jnp.int32(0x7FFFFFFF), bits)
        tok = lax.broadcasted_iota(i32, (OC, 1), 0) + r0
        key = ((key & jnp.int32(-S)) | (S - 1 - tok)).reshape(OC // 8, 8, 1)
        b1 = jnp.max(key, axis=0)
        b2 = jnp.max(jnp.where(key == b1, imin, key), axis=0)
        best2 = jnp.maximum(jnp.minimum(best1, b1), jnp.maximum(best2, b2))
        best1 = jnp.maximum(best1, b1)
        marks.append(best2)
        for j, (_, b) in enumerate(OUT_GROUPS):
            if b == r0 + OC:
                o_cp[j].start()
        attn = nxt

    k1 = jnp.max(best1)
    k2 = jnp.max(jnp.where(best1 == k1, best2, best1))
    i1 = S - 1 - (k1 & (S - 1))
    i2 = S - 1 - (k2 & (S - 1))
    row = lax.broadcasted_iota(i32, (16, D), 0)
    xsel = jnp.where(row == 0, ln2_v[pl.ds(i1, 1), :], ln2_v[pl.ds(i2, 1), :])
    gate = jax.nn.sigmoid(jnp.sum(xsel * wr, axis=-1, keepdims=True))
    xsel = xsel.astype(bf16)
    g = jnp.dot(xsel, wg_v[...], preferred_element_type=f32)
    u = jnp.dot(xsel, wu_v[...], preferred_element_type=f32)
    act = (g * jax.nn.sigmoid(g) * u).astype(bf16)
    y = jnp.dot(act, wd_v[...], preferred_element_type=f32) * gate
    fix = []
    for j, idx in enumerate((i1, i2)):
        b0 = pl.multiple_of((idx // 16) * 16, 16)
        upd = jnp.where(row + b0 == i1, y[0:1], 0.0) + jnp.where(row + b0 == i2, y[1:2], 0.0)
        fix_v[j] = (base_v[pl.ds(b0, 16), :] + upd).astype(bf16)
        fix.append(pltpu.make_async_copy(fix_v.at[j], out_hbm.at[pl.ds(b0, 16)], sem_o.at[j]))
    for cp in o_cp:
        cp.wait()
    fix[0].start()

    @pl.when(i1 // 16 != i2 // 16)
    def _():
        fix[1].start()
        fix[1].wait()

    fix[0].wait()


@jax.jit
def pallas_sequential_preLN__mha_block__moe_arch_mod__prompt_kernel(
    A_x: jax.Array,
    A_wqkv: jax.Array,
    A_wo: jax.Array,
    B_x: jax.Array,
    B_w_r: jax.Array,
    B_w_gate: jax.Array,
    B_w_up: jax.Array,
    B_w_down: jax.Array,
):
    del B_x
    any_spec = pl.BlockSpec(memory_space=pl.ANY)
    out = pl.pallas_call(
        _kernel,
        out_shape=jax.ShapeDtypeStruct((S, D), bf16),
        in_specs=[any_spec] * 7,
        out_specs=any_spec,
        scratch_shapes=[
            pltpu.VMEM((S, D), bf16),
            pltpu.VMEM((D, D), bf16),
            pltpu.VMEM((D, D), bf16),
            pltpu.VMEM((D, D), bf16),
            pltpu.VMEM((D, D), bf16),
            pltpu.VMEM((1, D), bf16),
            pltpu.VMEM((D, F), bf16),
            pltpu.VMEM((D, F), bf16),
            pltpu.VMEM((F, D), bf16),
            pltpu.VMEM((S, D), bf16),
            pltpu.VMEM((D // 2, D), u32),
            pltpu.VMEM((D // 2, D), u32),
            pltpu.VMEM((S // 2, D), u32),
            pltpu.VMEM((S, D), f32),
            pltpu.VMEM((16, S // 4, 128), u32),
            pltpu.VMEM((H * 32 + 16, S), u32),
            pltpu.VMEM((H, S), f32),
            pltpu.VMEM((D // 2, S), u32),
            pltpu.VMEM((8, TQ), f32),
            pltpu.VMEM((8, TQ), f32),
            pltpu.VMEM((D // 2, S), u32),
            pltpu.VMEM((1, TQ), f32),
            pltpu.VMEM((S, D), f32),
            pltpu.VMEM((S, D), f32),
            pltpu.VMEM((2, 16, D), bf16),
            pltpu.SMEM((1,), i32),
            pltpu.SemaphoreType.DMA((S // RC,)),
            pltpu.SemaphoreType.DMA((8,)),
            pltpu.SemaphoreType.DMA((len(OUT_GROUPS),)),
        ] + [pltpu.VMEM((PK // 2, TQ), u32)] * (2 * (S // PK)),
        compiler_params=pltpu.CompilerParams(vmem_limit_bytes=100 * 1024 * 1024),
    )(A_x.reshape(S, D), A_wqkv, A_wo, B_w_r.reshape(1, D), B_w_gate, B_w_up, B_w_down)
    return out.reshape(1, S, D)
```

```python
import functools

import jax
import jax.numpy as jnp
from jax import lax
import jax.experimental.pallas as pl
import jax.experimental.pallas.tpu as pltpu

S = 2048
D = 512
H = 32
DH = 16
F = 1792
EPS = 1e-5
QSCALE = (DH ** -0.5) * 1.4426950408889634

TQ = 512
KC = 256
PK = 512
NIT = H * (S // TQ)
UN = 14
LAG = 4
RC = 256
LNR = 64
TC = 128
OC = 128
OUT_GROUPS = ((0, 1024), (1024, 1792), (1792, 2048))

L_MIN = 2.0 ** -60
QK_MAX = 20.0
MAGIC = 12582912.0

bf16 = jnp.bfloat16
f32 = jnp.float32
u32 = jnp.uint32
i32 = jnp.int32
i8 = jnp.int8


def _tobf(x):
    return pltpu.bitcast(x, bf16)


def _toi8(x):
    return pltpu.bitcast(x, i8)


def _tou(x):
    return pltpu.bitcast(x, u32)


def _ln_stats(x):
    m = jnp.sum(x, axis=-1, keepdims=True) * (1.0 / D)
    ms = jnp.sum(x * x, axis=-1, keepdims=True) * (1.0 / D)
    return m, lax.rsqrt(jnp.maximum(ms - m * m, 0.0) + EPS)


def _limbs(t):
    hi = t + MAGIC
    lo = (t - (hi - MAGIC)) * 16.0 + MAGIC
    top = t * 0.0625 + MAGIC
    return hi, lo, top


def _pack8(x):
    return _tou(pltpu.bitcast(x, i32).astype(i8))


_NT = (((1,), (1,)), ((), ()))
_TN = (((0,), (0,)), ((), ()))


def _kernel(x_hbm, wqkv_hbm, wo_hbm, wr_hbm, wg_hbm, wu_hbm, wd_hbm, out_hbm,
            x_v, wq_v, wk_v, wv_v, wo_v, wr_v, wg_v, wu_v, wd_v, out_v,
            wqt_v, wvt_v, ln_v, kf_v, k8_v, w8_v, a_v, vt_v, l0_v, l1_v, ot_v, lmin_v,
            base_v, ln2_v, fix_v, z_s, sem_x, sem_w, sem_o, *p_v):
    nxc = S // RC
    x_cp = [pltpu.make_async_copy(x_hbm.at[pl.ds(c * RC, RC)], x_v.at[pl.ds(c * RC, RC)], sem_x.at[c])
            for c in range(nxc)]
    w_cp = [pltpu.make_async_copy(src, dst, sem_w.at[i]) for i, (src, dst) in enumerate(
        [(wqkv_hbm.at[:, pl.ds(D, D)], wk_v), (wqkv_hbm.at[:, pl.ds(0, D)], wq_v),
         (wqkv_hbm.at[:, pl.ds(2 * D, D)], wv_v),
         (wo_hbm, wo_v), (wr_hbm, wr_v), (wg_hbm, wg_v), (wu_hbm, wu_v), (wd_hbm, wd_v)])]
    x_cp[0].start()
    w_cp[0].start()
    for cp in x_cp[1:] + w_cp[1:]:
        cp.start()
    z_s[0] = 0

    def ln_rows(r0, n):
        for r in range(r0, r0 + n, LNR):
            x = x_v[r:r + LNR, :].astype(f32)
            m, rs = _ln_stats(x)
            ln_v[r // 2:(r + LNR) // 2, :] = _tou(((x - m) * rs).astype(bf16))

    waits = {0: [x_cp[1]], 1: x_cp[2:4], 3: x_cp[4:], nxc - 2: w_cp[1:3]}
    x_cp[0].wait()
    ln_rows(0, RC)
    w_cp[0].wait()
    kmax = jnp.zeros((8, D), f32)
    for c in range(nxc):
        r0 = c * RC
        for cp in waits.get(c, []):
            cp.wait()
        kc = jnp.dot(_tobf(ln_v[r0 // 2:(r0 + RC) // 2, :]), wk_v[...], preferred_element_type=f32)
        kf_v[r0:r0 + RC, :] = kc
        kmax = jnp.maximum(kmax, jnp.max(jnp.abs(kc).reshape(RC // 8, 8, D), axis=0))
        for h in range(H + 1):
            w8_v[32 * h:32 * h + 16, r0:r0 + RC] = jnp.zeros((16, RC), u32)
        if c + 1 < nxc:
            ln_rows(r0 + RC, RC)
        else:
            wqt_v[...] = _tou(wq_v[...].astype(f32).T.astype(bf16))
            wvt_v[...] = _tou(wv_v[...].astype(f32).T.astype(bf16))
    kmax_row = jnp.max(kmax, axis=0, keepdims=True)
    kcol = jnp.broadcast_to(kmax_row, (128, D)).T
    khead = jnp.maximum(jnp.max(kcol.reshape(H, DH, 128), axis=1), 1e-30)
    kinv_col = jnp.broadcast_to((127.0 / khead)[:, None, :], (H, DH, 128)).reshape(D, 128)
    kinv_row = kinv_col.T[0:8, :]

    lane = lax.broadcasted_iota(i32, (8, 128), 1)
    odd16 = (lane & 16) != 0
    odd32 = (lane & 32) != 0
    umax = jnp.minimum(kmax_row * kinv_row + 1.0, 127.0).astype(i32).astype(u32) * jnp.uint32(0x01010101)
    um_e = [pltpu.roll(umax[:, g * 128:(g + 1) * 128], 16, 1) for g in range(4)]
    um_o = [pltpu.roll(umax[:, g * 128:(g + 1) * 128], 112, 1) for g in range(4)]
    never = z_s[0] != 0

    def k_limbs(r0, pace):
        for g in range(4):
            kinv = jnp.where(never, pace, kinv_row[:, g * 128:(g + 1) * 128])
            u = (kf_v[r0:r0 + 32, g * 128:(g + 1) * 128].reshape(4, 8, 128) * kinv).reshape(32, 128)
            hi, lo, top = [_pack8(t) for t in _limbs(u)]
            e1 = jnp.where(odd16, pltpu.roll(lo, 16, 1), hi)
            o1 = jnp.where(odd16, hi, pltpu.roll(lo, 112, 1))
            e2 = jnp.where(odd16, um_e[g], top)
            o2 = jnp.where(odd16, top, um_o[g])
            rs = pl.ds(r0 // 4, 8)
            k8_v[4 * g + 0, rs, :] = jnp.where(odd32, pltpu.roll(e2, 32, 1), e1)
            k8_v[4 * g + 1, rs, :] = jnp.where(odd32, e1, pltpu.roll(e2, 96, 1))
            k8_v[4 * g + 2, rs, :] = jnp.where(odd32, pltpu.roll(o2, 32, 1), o1)
            k8_v[4 * g + 3, rs, :] = jnp.where(odd32, o1, pltpu.roll(o2, 96, 1))

    def q_limbs(c, g, qt):
        cols = slice(c * TC, (c + 1) * TC)
        qs = [qt[j * DH:(j + 1) * DH] for j in range(8)]
        ms = [jnp.maximum(jnp.abs(q[0:8]), jnp.abs(q[8:16])) for q in qs]
        for sh in (4, 2, 1):
            ms = [jnp.maximum(m, pltpu.roll(m, sh, 0)) for m in ms]
        ms = [jnp.maximum(m, 1e-30) for m in ms]
        invs = [127.0 / m for m in ms]
        for j in range(8):
            h = 8 * g + j
            a_v[h:h + 1, cols] = ms[j][j:j + 1]
            t = qs[j] * jnp.concatenate([invs[j], invs[j]], axis=0)
            hi, lo, top = _limbs(t)
            neg = MAGIC - jnp.abs(t)
            x1 = [hi, top] if j % 2 == 0 else [top, hi]
            x2 = [lo, neg] if j % 2 == 0 else [neg, lo]
            blocks = x1 + x2 if (j // 2) % 2 == 0 else x2 + x1
            w8_v[32 * h + 16:32 * h + 32, cols] = _pack8(jnp.concatenate(blocks, axis=0))

    def proj_t(w_ref, g, c):
        ln = _tobf(ln_v[c * TC // 2:(c + 1) * TC // 2, :])
        return lax.dot_general(_tobf(w_ref[64 * g:64 * (g + 1), :]), ln, _NT, preferred_element_type=f32)

    todo = None
    for c in range(S // TC):
        for g in range(4):
            qt = proj_t(wqt_v, g, c)
            if todo is not None:
                todo()
            todo = functools.partial(q_limbs, c, g, qt)
        for g in range(4):
            vt = proj_t(wvt_v, g, c)
            todo()
            vt_v[64 * g:64 * (g + 1), c * TC:(c + 1) * TC] = _tou(vt.astype(bf16))
            todo = functools.partial(k_limbs, c * TC + g * 32, vt[0:8])
    todo()
    a_all = a_v[...] * jnp.concatenate([khead * (QSCALE / (127.0 * 127.0))] * (S // 128), axis=1)
    a_v[...] = a_all
    qk = jnp.max(a_all) * (127.0 * 127.0)

    lmin_v[...] = jnp.full(lmin_v.shape, 1.0, f32)
    for p_ref in p_v:
        p_ref[PK // 2:, :] = jnp.zeros((8, TQ), u32)
    nkb = S // PK
    bufs = [(p_v[:nkb], l0_v), (p_v[nkb:], l1_v)]
    hist = []

    def step(sit, pit, cur, prev):
        z = z_s[0]
        if sit is not None:
            h = sit % H
            hh = h % 8
            kidx = (h // 8) * 4 + (hh & 1) * 2 + ((hh >> 1) & 1)
            q0 = pl.multiple_of((sit // H) * TQ, TQ)
            w0 = pl.multiple_of(32 * h + jnp.where(hh >= 4, 0, 16), 16)
            a = a_v[pl.ds(h, 1), pl.ds(q0, TQ)]
            l = jnp.zeros((8, TQ), f32)
        if pit is not None:
            pr0 = pl.multiple_of((pit % H) * 8, 8)
            pq0 = pl.multiple_of((pit // H) * TQ, TQ)
            accs = [jnp.zeros((16, 128), f32) for _ in range(TQ // 128)]
        pv = [(kb, nb) for kb in range(nkb) for nb in range(TQ // 128)]
        per = len(pv) // (S // KC)
        for kc in range(S // KC):
            if sit is not None:
                kk = _toi8(k8_v[kidx, pl.ds(kc * KC // 4, KC // 4), :])
                w = w8_v[pl.ds(w0, 32), pl.ds(q0, TQ)]
                if len(hist) >= LAG:
                    dep = _tou(hist[-LAG][0:8] + hist[-LAG + 1][0:8])
                    dep = jnp.concatenate([dep] * (TQ // 128), axis=1)
                    w = jnp.concatenate([w[0:24], jnp.where(z != 0, dep, w[24:32])], axis=0)
                s = jnp.dot(kk, _toi8(w), preferred_element_type=i32)
                p = jnp.exp2(s.astype(f32) * a)
                cur[0][kc * KC // PK][pl.ds((kc * KC % PK) // 2, KC // 2), :] = _tou(p.astype(bf16))
                l = l + jnp.sum(p.reshape(KC // 8, 8, TQ), axis=0)
            if pit is not None:
                for kb, nb in pv[kc * per:(kc + 1) * per]:
                    pt = _tobf(prev[0][kb][pl.ds(pl.multiple_of(z & 8, 8), PK // 2), pl.ds(nb * 128, 128)])
                    vt = _tobf(vt_v[pl.ds(pr0, 8), pl.ds(kb * PK, PK)])
                    res = jnp.dot(vt, pt, preferred_element_type=f32)
                    hist.append(res)
                    accs[nb] = accs[nb] + res
        if pit is not None:
            lsum = jnp.sum(prev[1][...], axis=0, keepdims=True)
            lmin_v[...] = jnp.minimum(lmin_v[...], lsum)
            o = jnp.concatenate(accs, axis=1) / lsum
            ot_v[pl.ds(pr0, 8), pl.ds(pq0, TQ)] = _tou(o.astype(bf16))
        if sit is not None:
            cur[1][...] = l

    npeel = (NIT - 1) % UN
    step(jnp.int32(0), None, bufs[0], None)
    for i in range(npeel):
        step(jnp.int32(i + 1), jnp.int32(i), bufs[(i + 1) % 2], bufs[i % 2])

    def body(it, carry):
        hist.clear()
        for u in range(npeel, npeel + UN):
            step(UN * it + u + 1, UN * it + u, bufs[(u + 1) % 2], bufs[u % 2])
        hist.clear()
        return carry

    lax.fori_loop(0, (NIT - 1) // UN, body, 0)
    step(None, jnp.int32(NIT - 1), None, bufs[(NIT - 1) % 2])

    ok = jnp.logical_and(jnp.min(lmin_v[...]) >= L_MIN, qk <= QK_MAX)

    @pl.when(jnp.logical_not(ok))
    def _():
        tf = 128

        def fb(it, carry):
            h = it % H
            r8 = pl.multiple_of(h * 8, 8)
            q0 = pl.multiple_of((it // H) * tf, tf)
            lnq = _tobf(ln_v[pl.ds(pl.multiple_of(q0 // 2, tf // 2), tf // 2), :])
            q16 = lax.dot_general(_tobf(wqt_v[pl.ds(r8, 8), :]), lnq, _NT, preferred_element_type=f32)
            q16 = _tou((q16 * QSCALE).astype(bf16))
            zero = jnp.zeros_like(q16)
            w = _tobf(jnp.concatenate([jnp.where(h % 8 == j, q16, zero) for j in range(8)], axis=0))
            kg = kf_v[:, pl.ds(pl.multiple_of((h // 8) * 128, 128), 128)].astype(bf16)
            s = jnp.dot(kg, w, preferred_element_type=f32)
            p = jnp.exp2(s - jnp.max(s, axis=0, keepdims=True))
            l = jnp.sum(p, axis=0, keepdims=True)
            o = jnp.dot(_tobf(vt_v[pl.ds(r8, 8), :]), p.astype(bf16), preferred_element_type=f32)
            ot_v[pl.ds(r8, 8), pl.ds(q0, tf)] = _tou((o / l).astype(bf16))
            return carry

        lax.fori_loop(0, H * (S // tf), fb, 0)

    for cp in w_cp[3:]:
        cp.wait()
    o_cp = [pltpu.make_async_copy(out_v.at[pl.ds(a, b - a)], out_hbm.at[pl.ds(a, b - a)], sem_o.at[j])
            for j, (a, b) in enumerate(OUT_GROUPS)]
    wr = wr_v[...].astype(f32)
    wr_sum = jnp.sum(wr, axis=-1, keepdims=True)
    imin = jnp.int32(-2 ** 31)
    marks = []

    def out_proj(c):
        ot = ot_v[:, c * OC:(c + 1) * OC]
        if c >= 3:
            dep = jnp.broadcast_to(_tou(marks[c - 3]), (8, OC))
            ot = jnp.concatenate([jnp.where(z_s[0] != 0, dep, ot[0:8]), ot[8:]], axis=0)
        return lax.dot_general(_tobf(ot), wo_v[...], _TN, preferred_element_type=f32)

    attn = out_proj(0)
    best1 = jnp.full((8, 1), imin, i32)
    best2 = jnp.full((8, 1), imin, i32)
    for c in range(S // OC):
        r0 = c * OC
        nxt = out_proj(c + 1) if r0 + OC < S else None
        h = x_v[r0:r0 + OC, :].astype(f32) + attn
        m, rs = _ln_stats(h)
        hw = jnp.sum(h * wr, axis=-1, keepdims=True)
        ln2 = (h - m) * rs
        base = h + ln2
        ln2_v[r0:r0 + OC, :] = ln2
        base_v[r0:r0 + OC, :] = base
        out_v[r0:r0 + OC, :] = base.astype(bf16)
        bits = pltpu.bitcast((hw - m * wr_sum) * rs, i32)
        key = jnp.where(bits < 0, bits ^ jnp.int32(0x7FFFFFFF), bits)
        tok = lax.broadcasted_iota(i32, (OC, 1), 0) + r0
        key = ((key & jnp.int32(-S)) | (S - 1 - tok)).reshape(OC // 8, 8, 1)
        b1 = jnp.max(key, axis=0)
        b2 = jnp.max(jnp.where(key == b1, imin, key), axis=0)
        best2 = jnp.maximum(jnp.minimum(best1, b1), jnp.maximum(best2, b2))
        best1 = jnp.maximum(best1, b1)
        marks.append(best2)
        for j, (_, b) in enumerate(OUT_GROUPS):
            if b == r0 + OC:
                o_cp[j].start()
        attn = nxt

    k1 = jnp.max(best1)
    k2 = jnp.max(jnp.where(best1 == k1, best2, best1))
    i1 = S - 1 - (k1 & (S - 1))
    i2 = S - 1 - (k2 & (S - 1))
    row = lax.broadcasted_iota(i32, (16, D), 0)
    xsel = jnp.where(row == 0, ln2_v[pl.ds(i1, 1), :], ln2_v[pl.ds(i2, 1), :])
    gate = jax.nn.sigmoid(jnp.sum(xsel * wr, axis=-1, keepdims=True))
    xsel = xsel.astype(bf16)
    g = jnp.dot(xsel, wg_v[...], preferred_element_type=f32)
    u = jnp.dot(xsel, wu_v[...], preferred_element_type=f32)
    act = (g * jax.nn.sigmoid(g) * u).astype(bf16)
    y = jnp.dot(act, wd_v[...], preferred_element_type=f32) * gate
    fix = []
    for j, idx in enumerate((i1, i2)):
        b0 = pl.multiple_of((idx // 16) * 16, 16)
        upd = jnp.where(row + b0 == i1, y[0:1], 0.0) + jnp.where(row + b0 == i2, y[1:2], 0.0)
        fix_v[j] = (base_v[pl.ds(b0, 16), :] + upd).astype(bf16)
        fix.append(pltpu.make_async_copy(fix_v.at[j], out_hbm.at[pl.ds(b0, 16)], sem_o.at[j]))
    for cp in o_cp:
        cp.wait()
    fix[0].start()

    @pl.when(i1 // 16 != i2 // 16)
    def _():
        fix[1].start()
        fix[1].wait()

    fix[0].wait()


@jax.jit
def pallas_sequential_preLN__mha_block__moe_arch_mod__prompt_kernel(
    A_x: jax.Array,
    A_wqkv: jax.Array,
    A_wo: jax.Array,
    B_x: jax.Array,
    B_w_r: jax.Array,
    B_w_gate: jax.Array,
    B_w_up: jax.Array,
    B_w_down: jax.Array,
):
    del B_x
    any_spec = pl.BlockSpec(memory_space=pl.ANY)
    out = pl.pallas_call(
        _kernel,
        out_shape=jax.ShapeDtypeStruct((S, D), bf16),
        in_specs=[any_spec] * 7,
        out_specs=any_spec,
        scratch_shapes=[
            pltpu.VMEM((S, D), bf16),
            pltpu.VMEM((D, D), bf16),
            pltpu.VMEM((D, D), bf16),
            pltpu.VMEM((D, D), bf16),
            pltpu.VMEM((D, D), bf16),
            pltpu.VMEM((1, D), bf16),
            pltpu.VMEM((D, F), bf16),
            pltpu.VMEM((D, F), bf16),
            pltpu.VMEM((F, D), bf16),
            pltpu.VMEM((S, D), bf16),
            pltpu.VMEM((D // 2, D), u32),
            pltpu.VMEM((D // 2, D), u32),
            pltpu.VMEM((S // 2, D), u32),
            pltpu.VMEM((S, D), f32),
            pltpu.VMEM((16, S // 4, 128), u32),
            pltpu.VMEM((H * 32 + 16, S), u32),
            pltpu.VMEM((H, S), f32),
            pltpu.VMEM((D // 2, S), u32),
            pltpu.VMEM((8, TQ), f32),
            pltpu.VMEM((8, TQ), f32),
            pltpu.VMEM((D // 2, S), u32),
            pltpu.VMEM((1, TQ), f32),
            pltpu.VMEM((S, D), f32),
            pltpu.VMEM((S, D), f32),
            pltpu.VMEM((2, 16, D), bf16),
            pltpu.SMEM((1,), i32),
            pltpu.SemaphoreType.DMA((S // RC,)),
            pltpu.SemaphoreType.DMA((8,)),
            pltpu.SemaphoreType.DMA((len(OUT_GROUPS),)),
        ] + [pltpu.VMEM((PK // 2 + 8, TQ), u32)] * (2 * (S // PK)),
        compiler_params=pltpu.CompilerParams(vmem_limit_bytes=100 * 1024 * 1024),
    )(A_x.reshape(S, D), A_wqkv, A_wo, B_w_r.reshape(1, D), B_w_gate, B_w_up, B_w_down)
    return out.reshape(1, S, D)
```

```python
import functools

import jax
import jax.numpy as jnp
from jax import lax
import jax.experimental.pallas as pl
import jax.experimental.pallas.tpu as pltpu

S = 2048
D = 512
H = 32
DH = 16
F = 1792
EPS = 1e-5
QSCALE = (DH ** -0.5) * 1.4426950408889634

TQ = 512
KC = 256
PK = 512
NIT = H * (S // TQ)
UN = 14
LAG = 4
XR = (128, 128) + (256,) * 7
LNR = 64
TC = 128
OC = 128
OUT_GROUPS = ((0, 1024), (1024, 1792), (1792, 2048))

L_MIN = 2.0 ** -60
QK_MAX = 20.0
MAGIC = 12582912.0

bf16 = jnp.bfloat16
f32 = jnp.float32
u32 = jnp.uint32
i32 = jnp.int32
i8 = jnp.int8


def _tobf(x):
    return pltpu.bitcast(x, bf16)


def _toi8(x):
    return pltpu.bitcast(x, i8)


def _tou(x):
    return pltpu.bitcast(x, u32)


def _ln_stats(x):
    m = jnp.sum(x, axis=-1, keepdims=True) * (1.0 / D)
    ms = jnp.sum(x * x, axis=-1, keepdims=True) * (1.0 / D)
    return m, lax.rsqrt(jnp.maximum(ms - m * m, 0.0) + EPS)


def _limbs(t):
    hi = t + MAGIC
    lo = (t - (hi - MAGIC)) * 16.0 + MAGIC
    top = t * 0.0625 + MAGIC
    return hi, lo, top


def _pack8(x):
    return _tou(pltpu.bitcast(x, i32).astype(i8))


_NT = (((1,), (1,)), ((), ()))
_TN = (((0,), (0,)), ((), ()))


def _kernel(x_hbm, wqkv_hbm, wo_hbm, wr_hbm, wg_hbm, wu_hbm, wd_hbm, out_hbm,
            x_v, wq_v, wk_v, wv_v, wo_v, wr_v, wg_v, wu_v, wd_v, out_v,
            wqt_v, wvt_v, ln_v, kf_v, k8_v, w8_v, a_v, vt_v, l0_v, l1_v, ot_v, lmin_v,
            base_v, ln2_v, fix_v, z_s, sem_x, sem_w, sem_o, *p_v):
    nxc = len(XR)
    xs = [sum(XR[:i]) for i in range(nxc + 1)]
    x_cp = [pltpu.make_async_copy(x_hbm.at[pl.ds(xs[c], XR[c])], x_v.at[pl.ds(xs[c], XR[c])], sem_x.at[c])
            for c in range(nxc)]
    w_cp = [pltpu.make_async_copy(src, dst, sem_w.at[i]) for i, (src, dst) in enumerate(
        [(wqkv_hbm.at[:, pl.ds(D, D)], wk_v), (wqkv_hbm.at[:, pl.ds(0, D)], wq_v),
         (wqkv_hbm.at[:, pl.ds(2 * D, D)], wv_v),
         (wo_hbm, wo_v), (wr_hbm, wr_v), (wg_hbm, wg_v), (wu_hbm, wu_v), (wd_hbm, wd_v)])]
    x_cp[0].start()
    w_cp[0].start()
    z_s[0] = 0

    def ln_rows(r0, n):
        for r in range(r0, r0 + n, LNR):
            x = x_v[r:r + LNR, :].astype(f32)
            m, rs = _ln_stats(x)
            ln_v[r // 2:(r + LNR) // 2, :] = _tou(((x - m) * rs).astype(bf16))

    starts = {0: x_cp[4:5], 1: x_cp[5:7], 2: x_cp[7:9], 3: w_cp[1:3], 7: w_cp[3:]}
    waits = {0: x_cp[1:2], 1: x_cp[2:3], 2: x_cp[3:5], 4: x_cp[5:9], 7: w_cp[1:3]}
    x_cp[0].wait()
    x_cp[1].start()
    x_cp[2].start()
    ln_rows(0, XR[0])
    w_cp[0].wait()
    x_cp[3].start()
    kmax = jnp.zeros((8, D), f32)
    for c in range(nxc):
        r0, n = xs[c], XR[c]
        for cp in waits.get(c, []):
            cp.wait()
        for cp in starts.get(c, []):
            cp.start()
        kc = jnp.dot(_tobf(ln_v[r0 // 2:(r0 + n) // 2, :]), wk_v[...], preferred_element_type=f32)
        kf_v[r0:r0 + n, :] = kc
        kmax = jnp.maximum(kmax, jnp.max(jnp.abs(kc).reshape(n // 8, 8, D), axis=0))
        if c + 1 < nxc:
            ln_rows(xs[c + 1], XR[c + 1])
        else:
            wqt_v[...] = _tou(wq_v[...].astype(f32).T.astype(bf16))
            wvt_v[...] = _tou(wv_v[...].astype(f32).T.astype(bf16))
    kmax_row = jnp.max(kmax, axis=0, keepdims=True)
    kcol = jnp.broadcast_to(kmax_row, (128, D)).T
    khead = jnp.maximum(jnp.max(kcol.reshape(H, DH, 128), axis=1), 1e-30)
    kinv_col = jnp.broadcast_to((127.0 / khead)[:, None, :], (H, DH, 128)).reshape(D, 128)
    kinv_row = kinv_col.T[0:8, :]

    lane = lax.broadcasted_iota(i32, (8, 128), 1)
    odd16 = (lane & 16) != 0
    odd32 = (lane & 32) != 0
    umax = jnp.minimum(kmax_row * kinv_row + 1.0, 127.0).astype(i32).astype(u32) * jnp.uint32(0x01010101)
    um_e = [pltpu.roll(umax[:, g * 128:(g + 1) * 128], 16, 1) for g in range(4)]
    um_o = [pltpu.roll(umax[:, g * 128:(g + 1) * 128], 112, 1) for g in range(4)]
    never = z_s[0] != 0

    def k_limbs(r0, pace):
        for g in range(4):
            kinv = jnp.where(never, pace, kinv_row[:, g * 128:(g + 1) * 128])
            u = (kf_v[r0:r0 + 32, g * 128:(g + 1) * 128].reshape(4, 8, 128) * kinv).reshape(32, 128)
            hi, lo, top = [_pack8(t) for t in _limbs(u)]
            e1 = jnp.where(odd16, pltpu.roll(lo, 16, 1), hi)
            o1 = jnp.where(odd16, hi, pltpu.roll(lo, 112, 1))
            e2 = jnp.where(odd16, um_e[g], top)
            o2 = jnp.where(odd16, top, um_o[g])
            rs = pl.ds(r0 // 4, 8)
            k8_v[4 * g + 0, rs, :] = jnp.where(odd32, pltpu.roll(e2, 32, 1), e1)
            k8_v[4 * g + 1, rs, :] = jnp.where(odd32, e1, pltpu.roll(e2, 96, 1))
            k8_v[4 * g + 2, rs, :] = jnp.where(odd32, pltpu.roll(o2, 32, 1), o1)
            k8_v[4 * g + 3, rs, :] = jnp.where(odd32, o1, pltpu.roll(o2, 96, 1))

    def q_limbs(c, g, qt):
        cols = slice(c * TC, (c + 1) * TC)
        qs = [qt[j * DH:(j + 1) * DH] for j in range(8)]
        ms = [jnp.maximum(jnp.abs(q[0:8]), jnp.abs(q[8:16])) for q in qs]
        for sh in (4, 2, 1):
            ms = [jnp.maximum(m, pltpu.roll(m, sh, 0)) for m in ms]
        ms = [jnp.maximum(m, 1e-30) for m in ms]
        invs = [127.0 / m for m in ms]
        for j in range(8):
            h = 8 * g + j
            a_v[h:h + 1, cols] = ms[j][j:j + 1]
            t = qs[j] * jnp.concatenate([invs[j], invs[j]], axis=0)
            hi, lo, top = _limbs(t)
            neg = MAGIC - jnp.abs(t)
            x1 = [hi, top] if j % 2 == 0 else [top, hi]
            x2 = [lo, neg] if j % 2 == 0 else [neg, lo]
            blocks = x1 + x2 if (j // 2) % 2 == 0 else x2 + x1
            w = _pack8(jnp.concatenate(blocks, axis=0))
            w8_v[32 * h + 16:32 * h + 32, cols] = w
            if j == 0:
                zero = jnp.where(never, w, jnp.uint32(0))
            w8_v[32 * h:32 * h + 16, cols] = zero
        if g == 3:
            w8_v[32 * H:, cols] = zero

    def proj_t(w_ref, g, c):
        ln = _tobf(ln_v[c * TC // 2:(c + 1) * TC // 2, :])
        return lax.dot_general(_tobf(w_ref[64 * g:64 * (g + 1), :]), ln, _NT, preferred_element_type=f32)

    todo = None
    for c in range(S // TC):
        for g in range(4):
            qt = proj_t(wqt_v, g, c)
            if todo is not None:
                todo()
            todo = functools.partial(q_limbs, c, g, qt)
        for g in range(4):
            vt = proj_t(wvt_v, g, c)
            todo()
            vt_v[64 * g:64 * (g + 1), c * TC:(c + 1) * TC] = _tou(vt.astype(bf16))
            todo = functools.partial(k_limbs, c * TC + g * 32, vt[0:8])
    todo()
    a_all = a_v[...] * jnp.concatenate([khead * (QSCALE / (127.0 * 127.0))] * (S // 128), axis=1)
    a_v[...] = a_all
    qk = jnp.max(a_all) * (127.0 * 127.0)

    lmin_v[...] = jnp.full(lmin_v.shape, 1.0, f32)
    for p_ref in p_v:
        p_ref[PK // 2:, :] = jnp.zeros((8, TQ), u32)
    nkb = S // PK
    bufs = [(p_v[:nkb], l0_v), (p_v[nkb:], l1_v)]
    hist = []

    def step(sit, pit, cur, prev):
        z = z_s[0]
        if sit is not None:
            h = sit % H
            hh = h % 8
            kidx = (h // 8) * 4 + (hh & 1) * 2 + ((hh >> 1) & 1)
            q0 = pl.multiple_of((sit // H) * TQ, TQ)
            w0 = pl.multiple_of(32 * h + jnp.where(hh >= 4, 0, 16), 16)
            a = a_v[pl.ds(h, 1), pl.ds(q0, TQ)]
            l = jnp.zeros((8, TQ), f32)
        if pit is not None:
            pr0 = pl.multiple_of((pit % H) * 8, 8)
            pq0 = pl.multiple_of((pit // H) * TQ, TQ)
            accs = [jnp.zeros((16, 128), f32) for _ in range(TQ // 128)]
        pv = [(kb, nb) for kb in range(nkb) for nb in range(TQ // 128)]
        per = len(pv) // (S // KC)
        for kc in range(S // KC):
            if sit is not None:
                kk = _toi8(k8_v[kidx, pl.ds(kc * KC // 4, KC // 4), :])
                w = w8_v[pl.ds(w0, 32), pl.ds(q0, TQ)]
                if len(hist) >= LAG:
                    dep = _tou(hist[-LAG][0:8] + hist[-LAG + 1][0:8])
                    dep = jnp.concatenate([dep] * (TQ // 128), axis=1)
                    w = jnp.concatenate([w[0:24], jnp.where(z != 0, dep, w[24:32])], axis=0)
                s = jnp.dot(kk, _toi8(w), preferred_element_type=i32)
                p = jnp.exp2(s.astype(f32) * a)
                cur[0][kc * KC // PK][pl.ds((kc * KC % PK) // 2, KC // 2), :] = _tou(p.astype(bf16))
                l = l + jnp.sum(p.reshape(KC // 8, 8, TQ), axis=0)
            if pit is not None:
                for kb, nb in pv[kc * per:(kc + 1) * per]:
                    pt = _tobf(prev[0][kb][pl.ds(pl.multiple_of(z & 8, 8), PK // 2), pl.ds(nb * 128, 128)])
                    vt = _tobf(vt_v[pl.ds(pr0, 8), pl.ds(kb * PK, PK)])
                    res = jnp.dot(vt, pt, preferred_element_type=f32)
                    hist.append(res)
                    accs[nb] = accs[nb] + res
        if pit is not None:
            lsum = jnp.sum(prev[1][...], axis=0, keepdims=True)
            lmin_v[...] = jnp.minimum(lmin_v[...], lsum)
            o = jnp.concatenate(accs, axis=1) / lsum
            ot_v[pl.ds(pr0, 8), pl.ds(pq0, TQ)] = _tou(o.astype(bf16))
        if sit is not None:
            cur[1][...] = l

    npeel = (NIT - 1) % UN
    step(jnp.int32(0), None, bufs[0], None)
    for i in range(npeel):
        step(jnp.int32(i + 1), jnp.int32(i), bufs[(i + 1) % 2], bufs[i % 2])

    def body(it, carry):
        hist.clear()
        for u in range(npeel, npeel + UN):
            step(UN * it + u + 1, UN * it + u, bufs[(u + 1) % 2], bufs[u % 2])
        hist.clear()
        return carry

    lax.fori_loop(0, (NIT - 1) // UN, body, 0)
    step(None, jnp.int32(NIT - 1), None, bufs[(NIT - 1) % 2])

    ok = jnp.logical_and(jnp.min(lmin_v[...]) >= L_MIN, qk <= QK_MAX)

    @pl.when(jnp.logical_not(ok))
    def _():
        tf = 128

        def fb(it, carry):
            h = it % H
            r8 = pl.multiple_of(h * 8, 8)
            q0 = pl.multiple_of((it // H) * tf, tf)
            lnq = _tobf(ln_v[pl.ds(pl.multiple_of(q0 // 2, tf // 2), tf // 2), :])
            q16 = lax.dot_general(_tobf(wqt_v[pl.ds(r8, 8), :]), lnq, _NT, preferred_element_type=f32)
            q16 = _tou((q16 * QSCALE).astype(bf16))
            zero = jnp.zeros_like(q16)
            w = _tobf(jnp.concatenate([jnp.where(h % 8 == j, q16, zero) for j in range(8)], axis=0))
            kg = kf_v[:, pl.ds(pl.multiple_of((h // 8) * 128, 128), 128)].astype(bf16)
            s = jnp.dot(kg, w, preferred_element_type=f32)
            p = jnp.exp2(s - jnp.max(s, axis=0, keepdims=True))
            l = jnp.sum(p, axis=0, keepdims=True)
            o = jnp.dot(_tobf(vt_v[pl.ds(r8, 8), :]), p.astype(bf16), preferred_element_type=f32)
            ot_v[pl.ds(r8, 8), pl.ds(q0, tf)] = _tou((o / l).astype(bf16))
            return carry

        lax.fori_loop(0, H * (S // tf), fb, 0)

    for cp in w_cp[3:]:
        cp.wait()
    o_cp = [pltpu.make_async_copy(out_v.at[pl.ds(a, b - a)], out_hbm.at[pl.ds(a, b - a)], sem_o.at[j])
            for j, (a, b) in enumerate(OUT_GROUPS)]
    wr = wr_v[...].astype(f32)
    wr_sum = jnp.sum(wr, axis=-1, keepdims=True)
    imin = jnp.int32(-2 ** 31)
    marks = []

    def out_proj(c):
        ot = ot_v[:, c * OC:(c + 1) * OC]
        if c >= 3:
            dep = jnp.broadcast_to(_tou(marks[c - 3]), (8, OC))
            ot = jnp.concatenate([jnp.where(z_s[0] != 0, dep, ot[0:8]), ot[8:]], axis=0)
        return lax.dot_general(_tobf(ot), wo_v[...], _TN, preferred_element_type=f32)

    attn = out_proj(0)
    best1 = jnp.full((8, 1), imin, i32)
    best2 = jnp.full((8, 1), imin, i32)
    for c in range(S // OC):
        r0 = c * OC
        nxt = out_proj(c + 1) if r0 + OC < S else None
        h = x_v[r0:r0 + OC, :].astype(f32) + attn
        m, rs = _ln_stats(h)
        hw = jnp.sum(h * wr, axis=-1, keepdims=True)
        ln2 = (h - m) * rs
        base = h + ln2
        ln2_v[r0:r0 + OC, :] = ln2
        base_v[r0:r0 + OC, :] = base
        out_v[r0:r0 + OC, :] = base.astype(bf16)
        bits = pltpu.bitcast((hw - m * wr_sum) * rs, i32)
        key = jnp.where(bits < 0, bits ^ jnp.int32(0x7FFFFFFF), bits)
        tok = lax.broadcasted_iota(i32, (OC, 1), 0) + r0
        key = ((key & jnp.int32(-S)) | (S - 1 - tok)).reshape(OC // 8, 8, 1)
        b1 = jnp.max(key, axis=0)
        b2 = jnp.max(jnp.where(key == b1, imin, key), axis=0)
        best2 = jnp.maximum(jnp.minimum(best1, b1), jnp.maximum(best2, b2))
        best1 = jnp.maximum(best1, b1)
        marks.append(best2)
        for j, (_, b) in enumerate(OUT_GROUPS):
            if b == r0 + OC:
                o_cp[j].start()
        attn = nxt

    k1 = jnp.max(best1)
    k2 = jnp.max(jnp.where(best1 == k1, best2, best1))
    i1 = S - 1 - (k1 & (S - 1))
    i2 = S - 1 - (k2 & (S - 1))
    row = lax.broadcasted_iota(i32, (16, D), 0)
    xsel = jnp.where(row == 0, ln2_v[pl.ds(i1, 1), :], ln2_v[pl.ds(i2, 1), :])
    gate = jax.nn.sigmoid(jnp.sum(xsel * wr, axis=-1, keepdims=True))
    xsel = xsel.astype(bf16)
    g = jnp.dot(xsel, wg_v[...], preferred_element_type=f32)
    u = jnp.dot(xsel, wu_v[...], preferred_element_type=f32)
    act = (g * jax.nn.sigmoid(g) * u).astype(bf16)
    y = jnp.dot(act, wd_v[...], preferred_element_type=f32) * gate
    fix = []
    for j, idx in enumerate((i1, i2)):
        b0 = pl.multiple_of((idx // 16) * 16, 16)
        upd = jnp.where(row + b0 == i1, y[0:1], 0.0) + jnp.where(row + b0 == i2, y[1:2], 0.0)
        fix_v[j] = (base_v[pl.ds(b0, 16), :] + upd).astype(bf16)
        fix.append(pltpu.make_async_copy(fix_v.at[j], out_hbm.at[pl.ds(b0, 16)], sem_o.at[j]))
    for cp in o_cp:
        cp.wait()
    fix[0].start()

    @pl.when(i1 // 16 != i2 // 16)
    def _():
        fix[1].start()
        fix[1].wait()

    fix[0].wait()


@jax.jit
def pallas_sequential_preLN__mha_block__moe_arch_mod__prompt_kernel(
    A_x: jax.Array,
    A_wqkv: jax.Array,
    A_wo: jax.Array,
    B_x: jax.Array,
    B_w_r: jax.Array,
    B_w_gate: jax.Array,
    B_w_up: jax.Array,
    B_w_down: jax.Array,
):
    del B_x
    any_spec = pl.BlockSpec(memory_space=pl.ANY)
    out = pl.pallas_call(
        _kernel,
        out_shape=jax.ShapeDtypeStruct((S, D), bf16),
        in_specs=[any_spec] * 7,
        out_specs=any_spec,
        scratch_shapes=[
            pltpu.VMEM((S, D), bf16),
            pltpu.VMEM((D, D), bf16),
            pltpu.VMEM((D, D), bf16),
            pltpu.VMEM((D, D), bf16),
            pltpu.VMEM((D, D), bf16),
            pltpu.VMEM((1, D), bf16),
            pltpu.VMEM((D, F), bf16),
            pltpu.VMEM((D, F), bf16),
            pltpu.VMEM((F, D), bf16),
            pltpu.VMEM((S, D), bf16),
            pltpu.VMEM((D // 2, D), u32),
            pltpu.VMEM((D // 2, D), u32),
            pltpu.VMEM((S // 2, D), u32),
            pltpu.VMEM((S, D), f32),
            pltpu.VMEM((16, S // 4, 128), u32),
            pltpu.VMEM((H * 32 + 16, S), u32),
            pltpu.VMEM((H, S), f32),
            pltpu.VMEM((D // 2, S), u32),
            pltpu.VMEM((8, TQ), f32),
            pltpu.VMEM((8, TQ), f32),
            pltpu.VMEM((D // 2, S), u32),
            pltpu.VMEM((1, TQ), f32),
            pltpu.VMEM((S, D), f32),
            pltpu.VMEM((S, D), f32),
            pltpu.VMEM((2, 16, D), bf16),
            pltpu.SMEM((1,), i32),
            pltpu.SemaphoreType.DMA((len(XR),)),
            pltpu.SemaphoreType.DMA((8,)),
            pltpu.SemaphoreType.DMA((len(OUT_GROUPS),)),
        ] + [pltpu.VMEM((PK // 2 + 8, TQ), u32)] * (2 * (S // PK)),
        compiler_params=pltpu.CompilerParams(vmem_limit_bytes=100 * 1024 * 1024),
    )(A_x.reshape(S, D), A_wqkv, A_wo, B_w_r.reshape(1, D), B_w_gate, B_w_up, B_w_down)
    return out.reshape(1, S, D)
```
